```python
import os as _os
_os.environ.setdefault("JAX_PLATFORMS", "cpu")
import jax
import jax.numpy as jnp

def _softmax(x, axis=-1):
    return jax.nn.softmax(x, axis=axis)
def _gelu(x):
    return jax.nn.gelu(x, approximate=True)
def _silu(x):
    return jax.nn.silu(x)
def _sigmoid(x):
    return jax.nn.sigmoid(x)
def _layernorm(x, axis=-1, eps=1e-5):
    m = jnp.mean(x, axis=axis, keepdims=True)
    v = jnp.var(x, axis=axis, keepdims=True)
    return (x - m) / jnp.sqrt(v + eps)
def _scatter_add(tgt, idx, src, axis=0):
    return tgt.at[idx].add(src)
def _segment_sum(src, seg, n):
    return jax.ops.segment_sum(src, seg, n)
class _Rng:
    def __init__(self, key):
        self._k = key
    def _next(self):
        self._k, sub = jax.random.split(self._k)
        return sub
    def normal(self, shape):
        return jax.random.normal(self._next(), shape, dtype=jnp.bfloat16)
    def randint(self, lo, hi, shape):
        return jax.random.randint(self._next(), shape, lo, hi, dtype=jnp.int32)
    def uniform(self, shape, lo=0.0, hi=1.0):
        return jax.random.uniform(self._next(), shape, jnp.bfloat16, lo, hi)
    def permutation(self, n):
        return jax.random.permutation(self._next(), n)


kernel_name = 'gated_mix__compressed_kv_cla__ssm_conv_h3__prompt'

def setup_inputs():
    _rng = _Rng(jax.random.key(int.from_bytes(__import__("os").urandom(4), "little")))
    _w = (lambda a: (lambda t: t.astype(jnp.bfloat16) if jnp.issubdtype(t.dtype, jnp.floating) else t)(jnp.asarray(a)))
    def _A_setup():
        B, H, Sq, Sk, D, M = 1, 32, 2048, 2048, 128, 1024
        Dc = 4 * D
        return {
            "x": _w((lambda *s: _rng.normal(s) * 0.05)(B, Sq, M)),
            "c_kv": _w((lambda *s: _rng.normal(s) * 0.8)(B, Sk, Dc)),
            "w_q": _w((lambda *s: _rng.normal(s) * 3.2)(M, H, D) * (M ** -0.5)),
            "w_uk": _w((lambda *s: _rng.normal(s) * 3.2)(Dc, H, D) * (Dc ** -0.5)),
            "w_uv": _w((lambda *s: _rng.normal(s) * 0.8)(Dc, H, D) * (Dc ** -0.5)),
            "w_o": _w((lambda *s: _rng.normal(s) * 0.8)(H, D, M) * ((H * D) ** -0.5)),
        }
    _A_in = _A_setup()

    def _B_setup():
        B, S, D = 1, 2048, 1024
        ks = 4
        return {
            "q": _w((lambda *s: _rng.normal(s) * 0.05)(B, S, D)),
            "k": _w((lambda *s: _rng.normal(s) * 0.8)(B, S, D)),
            "v": _w((lambda *s: _rng.normal(s) * 0.8)(B, S, D)),
            "shift_k": _w((lambda *s: _rng.normal(s) * 0.8)(D, ks) * 0.5),
            "ssm_k": _w((lambda *s: _rng.normal(s) * 0.8)(D, S) * (1.0 / S ** 0.5)),
            "ssm_D": _w((lambda *s: _rng.normal(s) * 0.8)(D)),
        }
    _B_in = _B_setup()

    return {
        "A_x": _A_in["x"],
        "A_c_kv": _A_in["c_kv"],
        "A_w_q": _A_in["w_q"],
        "A_w_uk": _A_in["w_uk"],
        "A_w_uv": _A_in["w_uv"],
        "A_w_o": _A_in["w_o"],
        "B_q": _B_in["q"],
        "B_k": _B_in["k"],
        "B_v": _B_in["v"],
        "B_shift_k": _B_in["shift_k"],
        "B_ssm_k": _B_in["ssm_k"],
        "B_ssm_D": _B_in["ssm_D"],
        "gate_w": _w((lambda *s: _rng.normal(s) * 0.05)(1024) * 16.0),
    }

def reference(A_x, A_c_kv, A_w_q, A_w_uk, A_w_uv, A_w_o, B_q, B_k, B_v, B_shift_k, B_ssm_k, B_ssm_D, gate_w):
    def _A_ref(x, c_kv, w_q, w_uk, w_uv, w_o):
        B, Sq, M = x.shape[0], x.shape[1], x.shape[2]
        Sk = c_kv.shape[1]
        H, D = w_q.shape[1], w_q.shape[2]
        q = jnp.einsum("bqm,mhd->bhqd", x, w_q)
        k = jnp.einsum("bkc,chd->bhkd", c_kv, w_uk)
        v = jnp.einsum("bkc,chd->bhkd", c_kv, w_uv)
        scores = jnp.einsum("bhqd,bhkd->bhqk", q, k) * (D ** -0.5)
        off = Sk - Sq
        qi = jnp.arange(Sq)[:, None]
        kj = jnp.arange(Sk)[None, :]
        cmask = kj <= (qi + off)
        scores = jnp.where(cmask[None, None], scores, -1e9)
        p = _softmax(scores, axis=-1)
        ctx = jnp.einsum("bhqk,bhkd->bhqd", p, v)
        return jnp.einsum("bhqd,hdm->bqm", ctx, w_o)

    def _B_ref(q, k, v, shift_k, ssm_k, ssm_D):
        B, S, D = q.shape
        ks = shift_k.shape[-1]
        k_pad = jnp.pad(k, ((0, 0), (ks - 1, 0), (0, 0)))
        k_shift = jnp.zeros_like(k)
        for t in range(ks):
            k_shift = k_shift + k_pad[:, t:t + S, :] * shift_k[:, ks - 1 - t][None, None, :]
        kv = k_shift * v
        L = 2 * S
        kv_pad = jnp.pad(kv, ((0, 0), (0, S), (0, 0)))
        kf_pad = jnp.pad(ssm_k, ((0, 0), (0, S)))
        kv_f = (lambda x, axes=(-2,-1): jnp.fft.rfft2(x.astype(jnp.float32), axes=axes))(kv_pad[:, None, :, :], axes=(1, 2))
        kf_f = (lambda x, axes=(-2,-1): jnp.fft.rfft2(x.astype(jnp.float32), axes=axes))(kf_pad[:, None, :], axes=(1, 2))
        kf_f = (lambda x, *d: x.transpose(*d))(kf_f, 1, 2, 0)
        y_f = kv_f * kf_f[None, :, :, :]
        y = (lambda x, s, axes=(-2,-1): jnp.fft.irfft2(x, s=s, axes=axes).astype(jnp.bfloat16))(y_f, (1, L), axes=(1, 2))[:, 0, :S, :]
        y = y + kv * ssm_D[None, None, :]
        return q * y

    x = A_x
    g = _sigmoid((x * gate_w).sum(-1, keepdims=True))
    a = _A_ref(x, A_c_kv, A_w_q, A_w_uk, A_w_uv, A_w_o)
    b = _B_ref(x, B_k, B_v, B_shift_k, B_ssm_k, B_ssm_D)
    return g * a + (1 - g) * b
```

```python
import functools
import math

import jax
import jax.numpy as jnp
from jax import lax
import jax.experimental.pallas as pl
import jax.experimental.pallas.tpu as pltpu

_F32 = jnp.float32
_BF16 = jnp.bfloat16
_NT = (((1,), (1,)), ((), ()))

_L = 128
_BQ = 512
_SB = 256
_CB = 128
_STRIP = 16
_RB = 256
_LSAFE = 2.0 ** 30


def _unpack_pair(u):
    lo = pltpu.bitcast(u << 16, _F32).astype(_BF16)
    hi = pltpu.bitcast(u & jnp.uint32(0xFFFF0000), _F32).astype(_BF16)
    return jnp.concatenate([lo, hi], axis=1)


def _qk_exp_off(q_ref, k_ref, p_ref, col, i):
    r0 = i * _BQ
    cs = slice(col, col + _L)
    lp = None
    for j0 in range(0, r0 // _L, 4):
        s = lax.dot_general(q_ref[r0:r0 + _BQ, cs], k_ref[j0 * _L:(j0 + 4) * _L, cs], _NT,
                            preferred_element_type=_F32)
        p = jnp.exp2(s)
        ps = [p[:, j * _L:(j + 1) * _L] for j in range(4)]
        t = (ps[0] + ps[1]) + (ps[2] + ps[3])
        lp = t if lp is None else lp + t
        ps[3] = jnp.minimum(ps[3], lp)
        p_ref[:, j0 * _L:(j0 + 4) * _L] = jnp.concatenate(ps, axis=1).astype(_BF16)
    return lp


def _qk_exp_diag(q_ref, k_ref, p_ref, col, i, cmask, lp):
    nd = _BQ // _L
    r0 = i * _BQ
    cs = slice(col, col + _L)
    lps = [None if lp is None else lp[r * _L:(r + 1) * _L] for r in range(nd)]
    for c in range(nd):
        c0 = r0 + c * _L
        sd = lax.dot_general(q_ref[c0:r0 + _BQ, cs], k_ref[c0:c0 + _L, cs], _NT,
                             preferred_element_type=_F32)
        p = jnp.exp2(sd)
        for r in range(c, nd):
            pr = p[(r - c) * _L:(r - c + 1) * _L]
            if r == c:
                pr = jnp.where(cmask, pr, 0.0)
            if lps[r] is None:
                lps[r] = pr
            else:
                lps[r] = lps[r] + pr
                pr = jnp.minimum(pr, lps[r])
            p_ref[r * _L:(r + 1) * _L, c0:c0 + _L] = pr.astype(_BF16)
    return lps


def _pv_off(p_ref, v_ref, col, i):
    r0 = i * _BQ
    if i == 0:
        return None
    return jnp.dot(p_ref[:, 0:r0], v_ref[0:r0, col:col + _L], preferred_element_type=_F32)


def _pv_diag(p_ref, v_ref, col, i):
    nd = _BQ // _L
    r0 = i * _BQ
    os_ = [None] * nd
    for c in range(nd):
        c0 = r0 + c * _L
        oc = jnp.dot(p_ref[c * _L:, c0:c0 + _L], v_ref[c0:c0 + _L, col:col + _L],
                     preferred_element_type=_F32)
        for r in range(c, nd):
            piece = oc[(r - c) * _L:(r - c + 1) * _L]
            os_[r] = piece if os_[r] is None else os_[r] + piece
    return os_


def _pv_finish(oo, os_, lps, o_ref, col, i, chk):
    r0 = i * _BQ
    for r in range(_BQ // _L):
        o = os_[r] if oo is None else os_[r] + oo[r * _L:(r + 1) * _L]
        l = jnp.sum(lps[r], axis=-1, keepdims=True)
        inv = pl.reciprocal(l, approx=True)
        inv = inv * (2.0 - l * inv)
        on = o * inv
        o_ref[r0 + r * _L:r0 + (r + 1) * _L, col:col + _L] = on.astype(o_ref.dtype)
        rng = (l + inv) + (on - on)
        chk = rng if chk is None else chk + rng
    return chk


def _kernel(x_hbm, c_hbm, wq_hbm, wk_hbm, wv_hbm, wo_hbm, bk_hbm, bv_hbm, ssmk_hbm,
            shift_ref, ssmd_ref, gw_ref,
            o_ref,
            x_s, c_s, wq_buf, wk_buf, wv_buf, wo_s, bk_s, bv_s, ssmk_s,
            sem_w, sem_in, sem_t,
            q_s, k_s, v_s, ctx_s, gate_s, gw_s, par_s, f_s, g_s, kp_s, chk_s,
            p_a, p_b, p_c, p_d, *, S, M, DC, H, D, KS):
    g = pl.program_id(0)
    n_pairs = H // 2
    n_ct = M // _L
    cb = _CB
    nb = S // cb
    nq = S // _BQ
    p_bufs = (p_a, p_b, p_c, p_d)
    qscale = (D ** -0.5) * math.log2(math.e)

    def w_copy(j, pair, slot):
        w, buf = ((wk_hbm, wk_buf), (wv_hbm, wv_buf), (wq_hbm, wq_buf))[j]
        return pltpu.make_async_copy(w.bitcast(jnp.uint32).at[:, pair, :], buf.at[slot],
                                     sem_w.at[j, slot])

    c_copy = pltpu.make_async_copy(c_hbm, c_s, sem_in.at[0])
    x_copy = pltpu.make_async_copy(x_hbm, x_s, sem_in.at[1])

    def tile_copies(c):
        cols = pl.ds(pl.multiple_of(c * _L, _L), _L)
        return [
            pltpu.make_async_copy(ssmk_hbm.at[cols, :], ssmk_s.at[c], sem_t.at[c, 0]),
            pltpu.make_async_copy(bk_hbm.at[:, cols], bk_s.at[c], sem_t.at[c, 1]),
            pltpu.make_async_copy(bv_hbm.at[:, cols], bv_s.at[c], sem_t.at[c, 2]),
            pltpu.make_async_copy(wo_hbm.at[:, cols], wo_s.at[c], sem_t.at[c, 3]),
        ]

    def proj(src_ref, w, dst_ref, i, scale=None):
        rsl = slice(i * _BQ, (i + 1) * _BQ)
        r = jnp.dot(src_ref[rsl, :], w, preferred_element_type=_F32)
        if scale is not None:
            r = r * scale
        dst_ref[rsl, :] = r.astype(_BF16)

    @pl.when(g == 0)
    def _init():
        w_copy(0, 0, 0).start()
        c_copy.start()
        w_copy(1, 0, 0).start()
        w_copy(2, 0, 0).start()
        x_copy.start()

        def dft(shape, raxis):
            r = lax.broadcasted_iota(jnp.int32, shape, raxis)
            t = lax.broadcasted_iota(jnp.int32, shape, 1 - raxis)
            part = r // cb
            rr = r % cb
            f = 2 * (rr % (cb // 2)) + rr // (cb // 2)
            k = ((2 * f + 1) * t + cb * part) % (4 * cb)
            return jnp.cos(k.astype(_F32) * (2.0 * math.pi / (4 * cb)))
        f_s[...] = dft((2 * cb, cb), 0).astype(_BF16)
        g_s[...] = (dft((cb, 2 * cb), 1) * (1.0 / cb)).astype(_BF16)
        gw_s[...] = jnp.broadcast_to(gw_ref[...].astype(_F32).reshape(1, M), (8, M))
        sh = shift_ref[...].astype(_F32)
        dd = ssmd_ref[...].astype(_F32).reshape(1, M)
        for c in range(n_ct):
            par_s[c, 0:KS, :] = sh[:, c * _L:(c + 1) * _L]
            par_s[c, KS:KS + 1, :] = dd[:, c * _L:(c + 1) * _L]
        kp_s[0:8, :] = jnp.zeros((8, _L), _F32)
        c_copy.wait()

    @pl.when(g < n_pairs)
    def _attention_step():
        slot = g % 2
        w_copy(0, g, slot).wait()
        w_copy(1, g, slot).wait()

        @pl.when(g > 0)
        def _():
            w_copy(2, g, slot).wait()

        @pl.when(jnp.logical_and(g > 0, g + 1 < n_pairs))
        def _():
            for j in range(3):
                w_copy(j, g + 1, 1 - slot).start()

        @pl.when(jnp.logical_and(g > 0, g <= n_ct))
        def _():
            for cp in tile_copies(g - 1):
                cp.start()

        wk = _unpack_pair(wk_buf[slot])
        wv = _unpack_pair(wv_buf[slot])
        for i in range(nq):
            proj(c_s, wk, k_s, i)
        for i in range(nq):
            proj(c_s, wv, v_s, i)

        @pl.when(g == 0)
        def _():
            w_copy(2, 0, 0).wait()
            x_copy.wait()
            for j in range(3):
                w_copy(j, 1, 1).start()

        rows = S // n_pairs
        rs = pl.ds(pl.multiple_of(g * rows, rows), rows)
        gl = jnp.sum(x_s[rs, :].astype(_F32) * gw_s[0:1, :], axis=-1, keepdims=True)
        gate_s[rs, :] = jnp.broadcast_to(jax.nn.sigmoid(gl), (rows, _L))

        wq = _unpack_pair(wq_buf[slot])
        row = lax.broadcasted_iota(jnp.int32, (_L, _L), 0)
        colid = lax.broadcasted_iota(jnp.int32, (_L, _L), 1)
        cmask = colid <= row
        ctx = ctx_s.at[g]

        def pv(i, lps, chk):
            pa, pb = p_bufs[2 * (i % 2)], p_bufs[2 * (i % 2) + 1]
            oa = _pv_off(pa, v_s, 0, i)
            ob = _pv_off(pb, v_s, D, i)
            da = _pv_diag(pa, v_s, 0, i)
            db = _pv_diag(pb, v_s, D, i)
            chk = _pv_finish(oa, da, lps[0], ctx, 0, i, chk)
            return _pv_finish(ob, db, lps[1], ctx, D, i, chk)

        chk = None
        pending = None
        for i in range(nq - 1, -1, -1):
            pa, pb = p_bufs[2 * (i % 2)], p_bufs[2 * (i % 2) + 1]
            proj(x_s, wq, q_s, i, qscale)
            if pending is not None:
                chk = pv(*pending, chk)
            la = _qk_exp_off(q_s, k_s, pa, 0, i)
            lb = _qk_exp_off(q_s, k_s, pb, D, i)
            la = _qk_exp_diag(q_s, k_s, pa, 0, i, cmask, la)
            lb = _qk_exp_diag(q_s, k_s, pb, D, i, cmask, lb)
            pending = (i, (la, lb))
        chk = pv(*pending, chk)
        bad = jnp.where(chk <= _LSAFE, 0.0, 1.0)
        b8 = bad[0:8]
        for r in range(1, _L // 8):
            b8 = jnp.maximum(b8, bad[r * 8:(r + 1) * 8])
        chk_s[g] = b8

    @pl.when(g == n_pairs)
    def _repair():
        def redo(p, carry):
            @pl.when(jnp.max(chk_s[p]) > 0.0)
            def _():
                for j in range(3):
                    w_copy(j, p, 0).start()
                for j in range(3):
                    w_copy(j, p, 0).wait()
                sb = _SB

                def pblock(i, c2):
                    rq = pl.ds(pl.multiple_of(i * sb, sb), sb)
                    for src, buf, dst, sc in ((c_s, wk_buf, k_s, 1.0), (c_s, wv_buf, v_s, 1.0),
                                              (x_s, wq_buf, q_s, qscale)):
                        r = jnp.dot(src[rq, :], _unpack_pair(buf[0]), preferred_element_type=_F32)
                        dst[rq, :] = (r * sc).astype(_BF16)
                    return c2

                lax.fori_loop(0, S // sb, pblock, 0)
                rid = lax.broadcasted_iota(jnp.int32, (sb, sb), 0)
                cid = lax.broadcasted_iota(jnp.int32, (sb, sb), 1)
                for h in range(2):
                    cs = slice(h * D, (h + 1) * D)

                    def qblock(i, c2):
                        rq = pl.ds(pl.multiple_of(i * sb, sb), sb)
                        q = q_s[rq, cs]

                        def kblock(j, st):
                            m, l, acc = st
                            rk = pl.ds(pl.multiple_of(j * sb, sb), sb)
                            s = lax.dot_general(q, k_s[rk, cs], _NT, preferred_element_type=_F32)
                            s = jnp.where(cid + j * sb <= rid + i * sb, s, -1e30)
                            m_new = jnp.maximum(m, jnp.max(s, axis=-1, keepdims=True))
                            alpha = jnp.exp2(m - m_new)
                            pm = jnp.exp2(s - m_new)
                            l = alpha * l + jnp.sum(pm, axis=-1, keepdims=True)
                            acc = alpha * acc + jnp.dot(pm.astype(_BF16), v_s[rk, cs],
                                                        preferred_element_type=_F32)
                            return m_new, l, acc

                        init = (jnp.full((sb, 1), -1e30, _F32), jnp.zeros((sb, 1), _F32),
                                jnp.zeros((sb, D), _F32))
                        m, l, acc = lax.fori_loop(0, i + 1, kblock, init)
                        ctx_s[p, rq, cs] = (acc / l).astype(_BF16)
                        return c2

                    lax.fori_loop(0, S // sb, qblock, 0)
            return carry

        anybad = chk_s[0]
        for p in range(1, n_pairs):
            anybad = jnp.maximum(anybad, chk_s[p])

        @pl.when(jnp.max(anybad) > 0.0)
        def _():
            lax.fori_loop(0, n_pairs, redo, 0)

    @pl.when(g >= n_pairs)
    def _output_step():
        c = g - n_pairs
        for cp in tile_copies(c):
            cp.wait()
        par = par_s[c, 0:KS + 1, :]
        L = _L
        half = cb // 2
        rb = _RB
        nchunks = S // rb
        nbef = 2
        wo = wo_s[c]

        def oproj(r):
            rsl = slice(r * rb, (r + 1) * rb)
            ctx = jnp.concatenate([ctx_s[p, rsl, :] for p in range(n_pairs)], axis=1)
            return jnp.dot(ctx, wo, preferred_element_type=_F32)

        fmat = f_s[...]
        hk = ssmk_s[c]
        hcat = jnp.concatenate([hk[:, m * cb:(m + 1) * cb] for m in range(nb)], axis=0)
        hh = lax.dot_general(fmat, hcat, _NT, preferred_element_type=_F32)
        kp_s[8:8 + S, :] = bk_s[c].astype(_F32)
        ksh = kp_s[8:8 + S, :] * par[0:1, :]
        for j in range(1, KS):
            ksh = ksh + kp_s[8 - j:8 - j + S, :] * par[j:j + 1, :]
        kv = (ksh * bv_s[c].astype(_F32)).astype(_BF16)
        acc, uhs = [], []
        gsz = nb // nbef
        for r in range(nbef):
            acc.append(oproj(r))
            ucat = jnp.concatenate([kv[i * cb:(i + 1) * cb, :]
                                    for i in range(r * gsz, (r + 1) * gsz)], axis=1)
            uhs.append(jnp.dot(fmat, ucat, preferred_element_type=_F32))
        uh = jnp.concatenate(uhs, axis=1)
        acc += [oproj(r) for r in range(nbef, nchunks - 1)]
        ua, ub, uab, hc, hdc, hcd = [], [], [], [], [], []
        for i in range(nb):
            re = uh[:cb, i * L:(i + 1) * L]
            im = uh[cb:, i * L:(i + 1) * L]
            if i > 0:
                pre = uh[:cb, (i - 1) * L:i * L]
                pim = uh[cb:, (i - 1) * L:i * L]
                re = jnp.concatenate([re[:half] - pim[:half], re[half:] + pim[half:]], axis=0)
                im = jnp.concatenate([im[:half] + pre[:half], im[half:] - pre[half:]], axis=0)
            ua.append(re)
            ub.append(im)
            uab.append(re + im)
            cre = hh[:cb, i * L:(i + 1) * L]
            cim = hh[cb:, i * L:(i + 1) * L]
            hc.append(cre)
            hdc.append(cim - cre)
            hcd.append(-cre - cim)
        sr = _STRIP
        yre = [[None] * (cb // sr) for _ in range(nb)]
        yim = [[None] * (cb // sr) for _ in range(nb)]
        tot = acc[nbef][rb - sr:, :] * 0.0
        for st in range(cb // sr):
            rs = slice(st * sr, (st + 1) * sr)
            for i in range(nb):
                marks = [tot]
                for hs, us in ((hdc, ua), (hc, uab), (hcd, ub)):
                    for m in range(i + 1):
                        tot = tot + hs[m][rs] * us[i - m][rs]
                    marks.append(tot)
                yim[i][st] = marks[2] - marks[0]
                yre[i][st] = marks[3] - marks[1]
        ys = [jnp.concatenate(yre[i] + yim[i], axis=0) for i in range(nb)]
        ycat = jnp.concatenate(ys, axis=1).astype(_BF16)
        yt = jnp.dot(g_s[...], ycat, preferred_element_type=_F32)
        acc.append(oproj(nchunks - 1))
        cols = pl.ds(pl.multiple_of(c * L, L), L)
        for r in range(nchunks):
            rsl = slice(r * rb, (r + 1) * rb)
            y = jnp.concatenate([yt[:, i * L:(i + 1) * L]
                                 for i in range(r * rb // cb, (r + 1) * rb // cb)], axis=0)
            y = y + kv[rsl, :].astype(_F32) * par[KS:KS + 1, :]
            b = x_s[rsl, cols].astype(_F32) * y
            gt = gate_s[rsl, :]
            o_ref[rsl, :] = (gt * acc[r] + (1.0 - gt) * b).astype(o_ref.dtype)


@jax.jit
def pallas_gated_mix__compressed_kv_cla__ssm_conv_h3__prompt_kernel(
    A_x: jax.Array,
    A_c_kv: jax.Array,
    A_w_q: jax.Array,
    A_w_uk: jax.Array,
    A_w_uv: jax.Array,
    A_w_o: jax.Array,
    B_q: jax.Array,
    B_k: jax.Array,
    B_v: jax.Array,
    B_shift_k: jax.Array,
    B_ssm_k: jax.Array,
    B_ssm_D: jax.Array,
    gate_w: jax.Array,
):
    del B_q
    B, S, M = A_x.shape
    DC = A_c_kv.shape[2]
    H, D = A_w_q.shape[1], A_w_q.shape[2]
    KS = B_shift_k.shape[1]
    assert B == 1 and D == _L and A_c_kv.shape[1] == S
    n_pairs = H // 2
    n_ct = M // _L
    assert n_ct < n_pairs

    hbm = pl.BlockSpec(memory_space=pl.ANY)
    in_specs = [hbm] * 9 + [
        pl.BlockSpec((KS, M), lambda g: (0, 0)),
        pl.BlockSpec((M,), lambda g: (0,)),
        pl.BlockSpec((M,), lambda g: (0,)),
    ]
    scratch = [
        pltpu.VMEM((S, M), _BF16),
        pltpu.VMEM((S, DC), _BF16),
        pltpu.VMEM((2, M, D), jnp.uint32),
        pltpu.VMEM((2, DC, D), jnp.uint32),
        pltpu.VMEM((2, DC, D), jnp.uint32),
        pltpu.VMEM((n_ct, H * D, _L), _BF16),
        pltpu.VMEM((n_ct, S, _L), _BF16),
        pltpu.VMEM((n_ct, S, _L), _BF16),
        pltpu.VMEM((n_ct, _L, S), _BF16),
        pltpu.SemaphoreType.DMA((3, 2)),
        pltpu.SemaphoreType.DMA((2,)),
        pltpu.SemaphoreType.DMA((n_ct, 4)),
        pltpu.VMEM((S, 2 * D), _BF16),
        pltpu.VMEM((S, 2 * D), _BF16),
        pltpu.VMEM((S, 2 * D), _BF16),
        pltpu.VMEM((n_pairs, S, 2 * D), _BF16),
        pltpu.VMEM((S, _L), _F32),
        pltpu.VMEM((8, M), _F32),
        pltpu.VMEM((n_ct, 8, _L), _F32),
        pltpu.VMEM((2 * _CB, _CB), _BF16),
        pltpu.VMEM((_CB, 2 * _CB), _BF16),
        pltpu.VMEM((S + 8, _L), _F32),
        pltpu.VMEM((n_pairs, 8, _L), _F32),
    ] + [pltpu.VMEM((_BQ, S), _BF16)] * 4
    out = pl.pallas_call(
        functools.partial(_kernel, S=S, M=M, DC=DC, H=H, D=D, KS=KS),
        grid=(n_pairs + n_ct,),
        in_specs=in_specs,
        out_specs=pl.BlockSpec((S, _L), lambda g: (0, jnp.maximum(g - n_pairs, 0))),
        out_shape=jax.ShapeDtypeStruct((S, M), A_x.dtype),
        scratch_shapes=scratch,
        compiler_params=pltpu.CompilerParams(
            dimension_semantics=("arbitrary",),
            vmem_limit_bytes=110 * 1024 * 1024,
        ),
    )(A_x.reshape(S, M), A_c_kv.reshape(S, DC), A_w_q, A_w_uk, A_w_uv,
      A_w_o.reshape(H * D, M), B_k.reshape(S, M), B_v.reshape(S, M), B_ssm_k,
      B_shift_k.T, B_ssm_D, gate_w)
    return out.reshape(B, S, M)
```

```python
import functools
import math

import jax
import jax.numpy as jnp
from jax import lax
import jax.experimental.pallas as pl
import jax.experimental.pallas.tpu as pltpu

_F32 = jnp.float32
_BF16 = jnp.bfloat16
_NT = (((1,), (1,)), ((), ()))

_L = 128
_BQ = 512
_HB = _BQ // 2
_SB = 256
_CB = 128
_STRIP = 16
_PG = 16
_RG = 32
_LSAFE = 2.0 ** 30


def _unpack_pair(u):
    return (pltpu.bitcast(u << 16, _F32), pltpu.bitcast(u & jnp.uint32(0xFFFF0000), _F32))


def _strassen_rhs_packed(buf, kh):
    def blk(r, c):
        u = buf[r * kh:(r + 1) * kh, :]
        u = (u << 16) if c == 0 else (u & jnp.uint32(0xFFFF0000))
        return pltpu.bitcast(u, _F32)
    return [blk(0, 0) + blk(1, 1), blk(0, 0), blk(0, 1) - blk(1, 1), blk(1, 0) - blk(0, 0),
            blk(1, 1), blk(0, 0) + blk(0, 1), blk(1, 0) + blk(1, 1)]


def _strassen_lhs(a11, a12, a21, a22):
    return [a11 + a22, a21 + a22, a11, a22, a11 + a12, a21 - a11, a12 - a22]


_SORDER = (4, 2, 6, 0, 3, 5, 1)


def _strassen_combine(m):
    c11 = ((m[6] - m[4]) + m[0]) + m[3]
    c12 = m[2] + m[4]
    c21 = m[3] + m[1]
    c22 = ((m[2] + m[0]) + m[5]) - m[1]
    return c11, c12, c21, c22


def _strassen(lhs, rhs):
    m = [None] * 7
    for j in _SORDER:
        m[j] = jnp.dot(lhs(j), rhs[j], preferred_element_type=_F32)
    return _strassen_combine(m)


def _qk_exp_off(q_ref, k_ref, p_ref, col, i):
    r0 = i * _BQ
    cs = slice(col, col + _L)
    lp = None
    for j0 in range(0, r0 // _L, 4):
        s = lax.dot_general(q_ref[r0:r0 + _BQ, cs], k_ref[j0 * _L:(j0 + 4) * _L, cs], _NT,
                            preferred_element_type=_F32)
        p = jnp.exp2(s)
        ps = [p[:, j * _L:(j + 1) * _L] for j in range(4)]
        t = (ps[0] + ps[1]) + (ps[2] + ps[3])
        lp = t if lp is None else lp + t
        p_ref[:, j0 * _L:(j0 + 4) * _L] = p.astype(_BF16)
    return lp


def _qk_exp_diag(q_ref, k_ref, p_ref, col, i, cmask, lp):
    nd = _BQ // _L
    r0 = i * _BQ
    cs = slice(col, col + _L)
    lps = [None if lp is None else lp[r * _L:(r + 1) * _L] for r in range(nd)]
    for c in range(nd):
        c0 = r0 + c * _L
        sd = lax.dot_general(q_ref[c0:r0 + _BQ, cs], k_ref[c0:c0 + _L, cs], _NT,
                             preferred_element_type=_F32)
        p = jnp.exp2(sd)
        for r in range(c, nd):
            pr = p[(r - c) * _L:(r - c + 1) * _L]
            if r == c:
                pr = jnp.where(cmask, pr, 0.0)
            lps[r] = pr if lps[r] is None else lps[r] + pr
            p_ref[r * _L:(r + 1) * _L, c0:c0 + _L] = pr.astype(_BF16)
    return lps


def _pv_off(p_ref, v_ref, col, i):
    r0 = i * _BQ
    if i == 0:
        return None
    return jnp.dot(p_ref[:, 0:r0], v_ref[0:r0, col:col + _L], preferred_element_type=_F32)


def _pv_diag(p_ref, v_ref, col, i):
    nd = _BQ // _L
    r0 = i * _BQ
    os_ = [None] * nd
    for c in range(nd):
        c0 = r0 + c * _L
        oc = jnp.dot(p_ref[c * _L:, c0:c0 + _L], v_ref[c0:c0 + _L, col:col + _L],
                     preferred_element_type=_F32)
        for r in range(c, nd):
            piece = oc[(r - c) * _L:(r - c + 1) * _L]
            os_[r] = piece if os_[r] is None else os_[r] + piece
    return os_


def _pv_norm(oo, os_, lps, chk):
    outs = []
    for r in range(_BQ // _L):
        o = os_[r] if oo is None else os_[r] + oo[r * _L:(r + 1) * _L]
        l = jnp.sum(lps[r], axis=-1, keepdims=True)
        inv = pl.reciprocal(l, approx=True)
        inv = inv * (2.0 - l * inv)
        on = o * inv
        outs.append(on)
        rng = (l + inv) + (on - on)
        chk = rng if chk is None else chk + rng
    return outs, chk


def _kernel(x_hbm, c_hbm, wq_hbm, wk_hbm, wv_hbm, wo_hbm, bk_hbm, bv_hbm, ssmk_hbm,
            shift_hbm, ssmd_hbm, gw_hbm,
            o_hbm,
            x_s, c_s, xs_s, cs_s, wq_buf, wk_buf, wv_buf, wo_s, bk_s, bv_s, ssmk_s,
            sem_w, sem_c, sem_x, sem_g, sem_o, olo_s, ohi_s, oa_s,
            q_s, k_s, v_s, ctx_s, gate_s, gw_s, par_s, f_s, g_s, kp_s, chk_s,
            a_s, b_s, p_a, p_b, p_c, p_d, shift_ref, ssmd_ref, gw_ref, *, S, M, DC, H, D, KS):
    g = pl.program_id(0)
    n_pairs = H // 2
    n_ct = M // _L
    cb = _CB
    nb = S // cb
    nq = S // _BQ
    hb = _HB
    ur = S // n_pairs
    p_bufs = (p_a, p_b, p_c, p_d)
    qscale = (D ** -0.5) * math.log2(math.e)

    def w_copy(j, pair, slot):
        w, buf = ((wk_hbm, wk_buf), (wv_hbm, wv_buf), (wq_hbm, wq_buf))[j]
        return pltpu.make_async_copy(w.bitcast(jnp.uint32).at[:, pair, :], buf.at[slot],
                                     sem_w.at[j, slot])

    def row_copy(src, dst, sem, i):
        rows = pl.ds(pl.multiple_of(i * _BQ, _BQ), _BQ)
        return pltpu.make_async_copy(src.at[rows, :], dst.at[rows, :], sem.at[i])

    def tile_copies(c):
        cols = pl.ds(pl.multiple_of(c * _L, _L), _L)
        return [
            pltpu.make_async_copy(ssmk_hbm.at[cols, :], ssmk_s.at[c], sem_g.at[0]),
            pltpu.make_async_copy(bk_hbm.at[:, cols], bk_s.at[c], sem_g.at[0]),
            pltpu.make_async_copy(bv_hbm.at[:, cols], bv_s.at[c], sem_g.at[0]),
            pltpu.make_async_copy(wo_hbm.at[:, cols], wo_s.at[c], sem_g.at[0]),
        ]

    def wait_and_sum(src_hbm, src_ref, sem, dst_ref, kh, after_wait=None):
        def body(i, carry):
            row_copy(src_hbm, src_ref, sem, i).wait()
            if after_wait is not None:
                after_wait(i)
            rg = _RG * (512 // kh)

            def inner(r, c2):
                rt = pl.ds(pl.multiple_of(i * _BQ + r * rg, rg), rg)
                rb_ = pl.ds(pl.multiple_of(i * _BQ + hb + r * rg, rg), rg)
                ro = pl.ds(pl.multiple_of(i * hb + r * rg, rg), rg)
                ops = _strassen_lhs(src_ref[rt, 0:kh].astype(_F32), src_ref[rt, kh:2 * kh].astype(_F32),
                                    src_ref[rb_, 0:kh].astype(_F32), src_ref[rb_, kh:2 * kh].astype(_F32))
                for n, j in enumerate((0, 1, 4, 5, 6)):
                    dst_ref[n, ro, :] = ops[j].astype(_BF16)
                return c2

            lax.fori_loop(0, hb // rg, inner, 0)
            return carry
        lax.fori_loop(0, nq, body, 0)

    def lhs_of(src_ref, sum_ref, kh, blocks):
        idx = {0: 0, 1: 1, 4: 2, 5: 3, 6: 4}

        def lhs(j):
            parts = []
            for i in blocks:
                if j == 2:
                    parts.append(src_ref[i * _BQ:i * _BQ + hb, 0:kh])
                elif j == 3:
                    parts.append(src_ref[i * _BQ + hb:(i + 1) * _BQ, kh:2 * kh])
                else:
                    parts.append(sum_ref[idx[j], i * hb:(i + 1) * hb, :])
            return jnp.concatenate(parts, axis=0) if len(parts) > 1 else parts[0]
        return lhs

    @pl.when(g == 0)
    def _init():
        w_copy(0, 0, 0).start()
        w_copy(1, 0, 0).start()
        for i in range(nq):
            row_copy(c_hbm, c_s, sem_c, i).start()
        small = [pltpu.make_async_copy(src, dst, sem_g.at[1]) for src, dst in (
            (shift_hbm, shift_ref), (ssmd_hbm, ssmd_ref), (gw_hbm, gw_ref))]
        for cp in small:
            cp.start()

        def dft(shape, raxis):
            r = lax.broadcasted_iota(jnp.int32, shape, raxis)
            t = lax.broadcasted_iota(jnp.int32, shape, 1 - raxis)
            part = r // cb
            rr = r % cb
            f = 2 * (rr % (cb // 2)) + rr // (cb // 2)
            k = ((2 * f + 1) * t + cb * part) % (4 * cb)
            return jnp.cos(k.astype(_F32) * (2.0 * math.pi / (4 * cb)))
        f_s[...] = dft((2 * cb, cb), 0).astype(_BF16)
        g_s[...] = (dft((cb, 2 * cb), 1) * (1.0 / cb)).astype(_BF16)
        kp_s[0:8, :] = jnp.zeros((8, _L), _F32)
        a_s[...] = jnp.zeros(a_s.shape, _F32)
        b_s[...] = jnp.zeros(b_s.shape, _F32)
        wait_and_sum(c_hbm, c_s, sem_c, cs_s, DC // 2,
                     lambda i: row_copy(x_hbm, x_s, sem_x, i).start())
        w_copy(2, 0, 0).start()
        for cp in small:
            cp.wait()
        gw_s[...] = jnp.broadcast_to(gw_ref[...].astype(_F32).reshape(1, M), (8, M))
        sh = shift_ref[...].astype(_F32)
        dd = ssmd_ref[...].astype(_F32).reshape(1, M)
        for c in range(n_ct):
            par_s[c, 0:KS, :] = sh[:, c * _L:(c + 1) * _L]
            par_s[c, KS:KS + 1, :] = dd[:, c * _L:(c + 1) * _L]

    @pl.when(g < n_pairs)
    def _attention_step():
        slot = g % 2
        w_copy(0, g, slot).wait()
        w_copy(1, g, slot).wait()

        @pl.when(g > 0)
        def _():
            w_copy(2, g, slot).wait()

        @pl.when(jnp.logical_and(g > 0, g + 1 < n_pairs))
        def _():
            for j in range(3):
                w_copy(j, g + 1, 1 - slot).start()

        @pl.when(jnp.logical_and(g > 0, g <= n_ct))
        def _():
            for cp in tile_copies(g - 1):
                cp.start()

        kh = DC // 2
        rkv = [jnp.concatenate([a, b], axis=1).astype(_BF16)
               for a, b in zip(_strassen_rhs_packed(wk_buf.at[slot], kh),
                               _strassen_rhs_packed(wv_buf.at[slot], kh))]
        c11, c12, c21, c22 = _strassen(lhs_of(c_s, cs_s, kh, range(nq)), rkv)
        for i in range(nq):
            rs_ = slice(i * hb, (i + 1) * hb)
            top = slice(i * _BQ, i * _BQ + hb)
            bot = slice(i * _BQ + hb, (i + 1) * _BQ)
            k_s[top, :] = jnp.concatenate([c11[rs_, :D], c12[rs_, :D]], axis=1).astype(_BF16)
            k_s[bot, :] = jnp.concatenate([c21[rs_, :D], c22[rs_, :D]], axis=1).astype(_BF16)
            v_s[top, :] = jnp.concatenate([c11[rs_, D:], c12[rs_, D:]], axis=1).astype(_BF16)
            v_s[bot, :] = jnp.concatenate([c21[rs_, D:], c22[rs_, D:]], axis=1).astype(_BF16)

        @pl.when(g == 0)
        def _():
            wait_and_sum(x_hbm, x_s, sem_x, xs_s, M // 2)
            w_copy(2, 0, 0).wait()
            for j in range(3):
                w_copy(j, 1, 1).start()

        rs = pl.ds(pl.multiple_of(g * ur, ur), ur)
        gl = jnp.sum(x_s[rs, :].astype(_F32) * gw_s[0:1, :], axis=-1, keepdims=True)
        gate_s[rs, :] = jnp.broadcast_to(jax.nn.sigmoid(gl), (ur, _L))

        mh = M // 2
        rq = [r.astype(_BF16) for r in _strassen_rhs_packed(wq_buf.at[slot], mh)]

        def qproj(i):
            c11, c12, c21, c22 = _strassen(lhs_of(x_s, xs_s, mh, [i]), rq)
            q_s[i * _BQ:i * _BQ + hb, :] = (jnp.concatenate([c11, c12], axis=1) * qscale).astype(_BF16)
            q_s[i * _BQ + hb:(i + 1) * _BQ, :] = (jnp.concatenate([c21, c22], axis=1) * qscale).astype(_BF16)

        row = lax.broadcasted_iota(jnp.int32, (_L, _L), 0)
        colid = lax.broadcasted_iota(jnp.int32, (_L, _L), 1)
        cmask = colid <= row

        def pv(i, lps, chk):
            pa, pb = p_bufs[2 * (i % 2)], p_bufs[2 * (i % 2) + 1]
            oa = _pv_off(pa, v_s, 0, i)
            ob = _pv_off(pb, v_s, D, i)
            da = _pv_diag(pa, v_s, 0, i)
            db = _pv_diag(pb, v_s, D, i)
            ca, chk = _pv_norm(oa, da, lps[0], chk)
            cb_, chk = _pv_norm(ob, db, lps[1], chk)
            ns = hb // _L
            for r in range(ns):
                ops = _strassen_lhs(ca[r], cb_[r], ca[r + ns], cb_[r + ns])
                for j in range(7):
                    ctx_s[j, g, i * hb + r * _L:i * hb + (r + 1) * _L, :] = ops[j].astype(_BF16)
            return chk

        chk = None
        pending = None
        for i in range(nq - 1, -1, -1):
            pa, pb = p_bufs[2 * (i % 2)], p_bufs[2 * (i % 2) + 1]
            qproj(i)
            if pending is not None:
                chk = pv(*pending, chk)
            la = _qk_exp_off(q_s, k_s, pa, 0, i)
            lb = _qk_exp_off(q_s, k_s, pb, D, i)
            la = _qk_exp_diag(q_s, k_s, pa, 0, i, cmask, la)
            lb = _qk_exp_diag(q_s, k_s, pb, D, i, cmask, lb)
            pending = (i, (la, lb))
        chk = pv(*pending, chk)
        bad = jnp.where(chk <= _LSAFE, 0.0, 1.0)
        b8 = bad[0:8]
        for r in range(1, _L // 8):
            b8 = jnp.maximum(b8, bad[r * 8:(r + 1) * 8])
        chk_s[g] = b8

    @pl.when(g == n_pairs)
    def _repair():
        for c in range(n_ct):
            for cp in tile_copies(c):
                cp.wait()

        def redo(p, carry):
            @pl.when(jnp.max(chk_s[p]) > 0.0)
            def _():
                for j in range(3):
                    w_copy(j, p, 0).start()
                for j in range(3):
                    w_copy(j, p, 0).wait()
                sb = _SB

                def pblock(i, c2):
                    rq = pl.ds(pl.multiple_of(i * sb, sb), sb)
                    for src, buf, dst, sc in ((c_s, wk_buf, k_s, 1.0), (c_s, wv_buf, v_s, 1.0),
                                              (x_s, wq_buf, q_s, qscale)):
                        w = jnp.concatenate(_unpack_pair(buf[0]), axis=1).astype(_BF16)
                        r = jnp.dot(src[rq, :], w, preferred_element_type=_F32)
                        dst[rq, :] = (r * sc).astype(_BF16)
                    return c2

                lax.fori_loop(0, S // sb, pblock, 0)
                rid = lax.broadcasted_iota(jnp.int32, (sb, sb), 0)
                cid = lax.broadcasted_iota(jnp.int32, (sb, sb), 1)
                for h in range(2):
                    cs = slice(h * D, (h + 1) * D)

                    def qblock(i, c2):
                        rq = pl.ds(pl.multiple_of(i * sb, sb), sb)
                        q = q_s[rq, cs]

                        def kblock(j, st):
                            m, l, acc = st
                            rk = pl.ds(pl.multiple_of(j * sb, sb), sb)
                            s = lax.dot_general(q, k_s[rk, cs], _NT, preferred_element_type=_F32)
                            s = jnp.where(cid + j * sb <= rid + i * sb, s, -1e30)
                            m_new = jnp.maximum(m, jnp.max(s, axis=-1, keepdims=True))
                            alpha = jnp.exp2(m - m_new)
                            pm = jnp.exp2(s - m_new)
                            l = alpha * l + jnp.sum(pm, axis=-1, keepdims=True)
                            acc = alpha * acc + jnp.dot(pm.astype(_BF16), v_s[rk, cs],
                                                        preferred_element_type=_F32)
                            return m_new, l, acc

                        init = (jnp.full((sb, 1), -1e30, _F32), jnp.zeros((sb, 1), _F32),
                                jnp.zeros((sb, D), _F32))
                        m, l, acc = lax.fori_loop(0, i + 1, kblock, init)
                        a_s[h, rq, :] = acc / l
                        return c2

                    lax.fori_loop(0, S // sb, qblock, 0)

                def cblock(i, c2):
                    rt = pl.ds(pl.multiple_of(i * _BQ, _BQ), hb)
                    rb_ = pl.ds(pl.multiple_of(i * _BQ + hb, hb), hb)
                    ro = pl.ds(pl.multiple_of(i * hb, hb), hb)
                    ops = _strassen_lhs(a_s[0, rt, :], a_s[1, rt, :], a_s[0, rb_, :], a_s[1, rb_, :])
                    for j in range(7):
                        ctx_s[j, p, ro, :] = ops[j].astype(_BF16)
                    return c2

                lax.fori_loop(0, nq, cblock, 0)
            return carry

        anybad = chk_s[0]
        for p in range(1, n_pairs):
            anybad = jnp.maximum(anybad, chk_s[p])

        @pl.when(jnp.max(anybad) > 0.0)
        def _():
            lax.fori_loop(0, n_pairs, redo, 0)

    @pl.when(g >= n_pairs)
    def _output_step():
        c = g - n_pairs
        n = c // 2
        mh = c % 2
        L = _L
        half = cb // 2
        nblk = nq // 2
        hs_ = S // 2

        def out_copy(nn, t, h):
            ocols = pl.ds(pl.multiple_of((nn * 2 + t) * L, L), L)
            if h == 0:
                src = olo_s.at[nn % 2, t]
            else:
                src = oa_s.at[nn % 2] if t == 0 else ohi_s.at[nn % 2]
            return pltpu.make_async_copy(src, o_hbm.at[h * hs_:(h + 1) * hs_, ocols], sem_o.at[nn % 2])

        def wait_out(nn):
            for t in range(2):
                for h in range(2):
                    out_copy(nn, t, h).wait()

        @pl.when(jnp.logical_and(mh == 0, n >= 2))
        def _():
            wait_out(n - 2)

        def wo_block(t, a):
            return jnp.concatenate([wo_s[2 * n + t, (2 * p + a) * D:(2 * p + a + 1) * D, :]
                                    for p in range(n_pairs)], axis=0)

        def wo_sum(x, y, sign):
            x, y = wo_block(*x).astype(_F32), wo_block(*y).astype(_F32)
            return (x + y if sign > 0 else x - y).astype(_BF16)

        b11, b12, b21, b22 = (0, 0), (1, 0), (0, 1), (1, 1)
        rhs = [wo_sum(b11, b22, 1), wo_block(*b11), wo_sum(b12, b22, -1), wo_sum(b21, b11, -1),
               wo_block(*b22), wo_sum(b11, b12, 1), wo_sum(b21, b22, 1)]
        prods = [[None] * 7 for _ in range(nblk)]
        todo = [(ii, j) for ii in range(nblk) for j in _SORDER]

        def oproj():
            ii, j = todo.pop(0)
            rows = pl.ds(pl.multiple_of((mh * nblk + ii) * hb, hb), hb)
            lhs = jnp.concatenate([ctx_s[j, p, rows, :] for p in range(n_pairs)], axis=1)
            prods[ii][j] = jnp.dot(lhs, rhs[j], preferred_element_type=_F32)
            return prods[ii][j]

        par = par_s[c, 0:KS + 1, :]
        kp_s[8:8 + S, :] = bk_s[c].astype(_F32)
        kvs = []
        tok = None
        p0 = jnp.broadcast_to(par[0:1, :], (_PG, L))
        for r in range(0, S, _PG):
            ksh = kp_s[8 + r:8 + r + _PG, :] * (p0 if tok is None else p0 + tok)
            for j in range(1, KS):
                ksh = ksh + kp_s[8 + r - j:8 + r - j + _PG, :] * par[j:j + 1, :]
            kvr = ksh * bv_s[c, r:r + _PG, :].astype(_F32)
            tok = kvr * 0.0
            kvs.append(kvr.astype(_BF16))
        kv = jnp.concatenate(kvs, axis=0)

        seq = 'OOHOUOHOUOT' + 'O' * (7 * nblk - 6) + 'I'
        nu = seq.count('U')
        nh = seq.count('H')
        fmat = f_s[...]
        hk = ssmk_s[c]
        uhs, hhs = [], []
        sr = _STRIP
        st = {}

        def conv():
            uh = jnp.concatenate(uhs, axis=1) if len(uhs) > 1 else uhs[0]
            hh = jnp.concatenate(hhs, axis=1) if len(hhs) > 1 else hhs[0]
            ua, ub, uab, hc, hdc, hcd = [], [], [], [], [], []
            for i in range(nb):
                re = uh[:cb, i * L:(i + 1) * L]
                im = uh[cb:, i * L:(i + 1) * L]
                if i > 0:
                    pre = uh[:cb, (i - 1) * L:i * L]
                    pim = uh[cb:, (i - 1) * L:i * L]
                    re = jnp.concatenate([re[:half] - pim[:half], re[half:] + pim[half:]], axis=0)
                    im = jnp.concatenate([im[:half] + pre[:half], im[half:] - pre[half:]], axis=0)
                ua.append(re)
                ub.append(im)
                uab.append(re + im)
                cre = hh[:cb, i * L:(i + 1) * L]
                cim = hh[cb:, i * L:(i + 1) * L]
                hc.append(cre)
                hdc.append(cim - cre)
                hcd.append(-cre - cim)
            yre = [[None] * (cb // sr) for _ in range(nb)]
            yim = [[None] * (cb // sr) for _ in range(nb)]
            tot = st['tot']
            for k in range(cb // sr):
                rs = slice(k * sr, (k + 1) * sr)
                for i in range(nb):
                    marks = [tot]
                    for hs, us in ((hdc, ua), (hc, uab), (hcd, ub)):
                        for m in range(i + 1):
                            tot = tot + hs[m][rs] * us[i - m][rs]
                        marks.append(tot)
                    yim[i][k] = marks[2] - marks[0]
                    yre[i][k] = marks[3] - marks[1]
            ys = [jnp.concatenate(yre[i] + yim[i], axis=0) for i in range(nb)]
            ycat = jnp.concatenate(ys, axis=1).astype(_BF16)
            return jnp.dot(g_s[...], ycat, preferred_element_type=_F32)

        for t in seq:
            if t == 'O':
                st['last'] = oproj()
            elif t == 'H':
                k, gs = len(hhs), nb // nh
                hcat = jnp.concatenate([hk[:, m * cb:(m + 1) * cb]
                                        for m in range(k * gs, (k + 1) * gs)], axis=0)
                hhs.append(lax.dot_general(fmat, hcat, _NT, preferred_element_type=_F32))
            elif t == 'U':
                k, gs = len(uhs), nb // nu
                ucat = jnp.concatenate([kv[i * cb:(i + 1) * cb, :]
                                        for i in range(k * gs, (k + 1) * gs)], axis=1)
                uhs.append(jnp.dot(fmat, ucat, preferred_element_type=_F32))
            elif t == 'T':
                st['tot'] = st['last'][hb - sr:, :] * 0.0
            elif t == 'I':
                yt = conv()
        assert not todo
        for ii in range(nblk):
            c11, c12, c21, c22 = _strassen_combine(prods[ii])
            r0 = (mh * nblk + ii) * _BQ
            top = pl.ds(pl.multiple_of(r0, _BQ), hb)
            bot = pl.ds(pl.multiple_of(r0 + hb, hb), hb)
            gt, gb = gate_s[top, :], gate_s[bot, :]
            c11, c21 = gt * c11, gb * c21
            a_s[0, top, :] = c11
            a_s[0, bot, :] = c21
            a_s[1, top, :] = gt * c12
            a_s[1, bot, :] = gb * c22
            lt, lb = slice(ii * _BQ, ii * _BQ + hb), slice(ii * _BQ + hb, (ii + 1) * _BQ)
            oa_s[n % 2, lt, :] = (c11 + b_s[lt, :]).astype(_BF16)
            oa_s[n % 2, lb, :] = (c21 + b_s[lb, :]).astype(_BF16)

        @pl.when(mh == 1)
        def _():
            out_copy(n, 0, 1).start()

        cols = pl.ds(pl.multiple_of(c * L, L), L)
        dd = par[KS:KS + 1, :]
        for i in range(nb):
            rsl = slice(i * cb, (i + 1) * cb)
            y = yt[:, i * L:(i + 1) * L] + kv[rsl, :].astype(_F32) * dd
            b = (1.0 - gate_s[rsl, :]) * (x_s[rsl, cols].astype(_F32) * y)
            o = (b + a_s[mh, rsl, :]).astype(_BF16)
            if i < nb // 2:
                olo_s[n % 2, mh, rsl, :] = o
            else:
                b_s[i * cb - hs_:(i + 1) * cb - hs_, :] = b
                ohi_s[n % 2, i * cb - hs_:(i + 1) * cb - hs_, :] = o
            if i == nb // 2 - 1:
                out_copy(n, mh, 0).start()

        @pl.when(mh == 1)
        def _():
            out_copy(n, 1, 1).start()

        @pl.when(c == n_ct - 1)
        def _():
            wait_out(n - 1)
            wait_out(n)


@jax.jit
def pallas_gated_mix__compressed_kv_cla__ssm_conv_h3__prompt_kernel(
    A_x: jax.Array,
    A_c_kv: jax.Array,
    A_w_q: jax.Array,
    A_w_uk: jax.Array,
    A_w_uv: jax.Array,
    A_w_o: jax.Array,
    B_q: jax.Array,
    B_k: jax.Array,
    B_v: jax.Array,
    B_shift_k: jax.Array,
    B_ssm_k: jax.Array,
    B_ssm_D: jax.Array,
    gate_w: jax.Array,
):
    del B_q
    B, S, M = A_x.shape
    DC = A_c_kv.shape[2]
    H, D = A_w_q.shape[1], A_w_q.shape[2]
    KS = B_shift_k.shape[1]
    assert B == 1 and D == _L and A_c_kv.shape[1] == S
    n_pairs = H // 2
    n_ct = M // _L
    nq = S // _BQ
    assert n_ct < n_pairs and n_ct % 2 == 0 and nq % 2 == 0 and KS < 8

    hbm = pl.BlockSpec(memory_space=pl.ANY)
    in_specs = [hbm] * 12
    scratch = [
        pltpu.VMEM((S, M), _BF16),
        pltpu.VMEM((S, DC), _BF16),
        pltpu.VMEM((5, S // 2, M // 2), _BF16),
        pltpu.VMEM((5, S // 2, DC // 2), _BF16),
        pltpu.VMEM((2, M, D), jnp.uint32),
        pltpu.VMEM((2, DC, D), jnp.uint32),
        pltpu.VMEM((2, DC, D), jnp.uint32),
        pltpu.VMEM((n_ct, H * D, _L), _BF16),
        pltpu.VMEM((n_ct, S, _L), _BF16),
        pltpu.VMEM((n_ct, S, _L), _BF16),
        pltpu.VMEM((n_ct, _L, S), _BF16),
        pltpu.SemaphoreType.DMA((3, 2)),
        pltpu.SemaphoreType.DMA((nq,)),
        pltpu.SemaphoreType.DMA((nq,)),
        pltpu.SemaphoreType.DMA((2,)),
        pltpu.SemaphoreType.DMA((2,)),
        pltpu.VMEM((2, 2, S // 2, _L), _BF16),
        pltpu.VMEM((2, S // 2, _L), _BF16),
        pltpu.VMEM((2, S // 2, _L), _BF16),
        pltpu.VMEM((S, 2 * D), _BF16),
        pltpu.VMEM((S, 2 * D), _BF16),
        pltpu.VMEM((S, 2 * D), _BF16),
        pltpu.VMEM((7, n_pairs, S // 2, D), _BF16),
        pltpu.VMEM((S, _L), _F32),
        pltpu.VMEM((8, M), _F32),
        pltpu.VMEM((n_ct, 8, _L), _F32),
        pltpu.VMEM((2 * _CB, _CB), _BF16),
        pltpu.VMEM((_CB, 2 * _CB), _BF16),
        pltpu.VMEM((S + 8, _L), _F32),
        pltpu.VMEM((n_pairs, 8, _L), _F32),
        pltpu.VMEM((2, S, _L), _F32),
        pltpu.VMEM((S // 2, _L), _F32),
    ] + [pltpu.VMEM((_BQ, S), _BF16)] * 4 + [
        pltpu.VMEM((KS, M), _BF16),
        pltpu.VMEM((M,), _BF16),
        pltpu.VMEM((M,), _BF16),
    ]
    out = pl.pallas_call(
        functools.partial(_kernel, S=S, M=M, DC=DC, H=H, D=D, KS=KS),
        grid=(n_pairs + n_ct,),
        in_specs=in_specs,
        out_specs=hbm,
        out_shape=jax.ShapeDtypeStruct((S, M), A_x.dtype),
        scratch_shapes=scratch,
        compiler_params=pltpu.CompilerParams(
            dimension_semantics=("arbitrary",),
            vmem_limit_bytes=120 * 1024 * 1024,
            disable_bounds_checks=True,
        ),
    )(A_x.reshape(S, M), A_c_kv.reshape(S, DC), A_w_q, A_w_uk, A_w_uv,
      A_w_o.reshape(H * D, M), B_k.reshape(S, M), B_v.reshape(S, M), B_ssm_k,
      B_shift_k.T, B_ssm_D, gate_w)
    return out.reshape(B, S, M)
```
